```python
import os as _os
_os.environ.setdefault("JAX_PLATFORMS", "cpu")
import jax
import jax.numpy as jnp

def _softmax(x, axis=-1):
    return jax.nn.softmax(x, axis=axis)
def _gelu(x):
    return jax.nn.gelu(x, approximate=True)
def _silu(x):
    return jax.nn.silu(x)
def _sigmoid(x):
    return jax.nn.sigmoid(x)
def _layernorm(x, axis=-1, eps=1e-5):
    m = jnp.mean(x, axis=axis, keepdims=True)
    v = jnp.var(x, axis=axis, keepdims=True)
    return (x - m) / jnp.sqrt(v + eps)
def _scatter_add(tgt, idx, src, axis=0):
    return tgt.at[idx].add(src)
def _segment_sum(src, seg, n):
    return jax.ops.segment_sum(src, seg, n)
class _Rng:
    def __init__(self, key):
        self._k = key
    def _next(self):
        self._k, sub = jax.random.split(self._k)
        return sub
    def normal(self, shape):
        return jax.random.normal(self._next(), shape, dtype=jnp.bfloat16)
    def randint(self, lo, hi, shape):
        return jax.random.randint(self._next(), shape, lo, hi, dtype=jnp.int32)
    def uniform(self, shape, lo=0.0, hi=1.0):
        return jax.random.uniform(self._next(), shape, jnp.bfloat16, lo, hi)
    def permutation(self, n):
        return jax.random.permutation(self._next(), n)


kernel_name = 'sequential_preLN__mha_block__dense_activation_mish__prompt'

def setup_inputs():
    _rng = _Rng(jax.random.key(int.from_bytes(__import__("os").urandom(4), "little")))
    _w = (lambda a: (lambda t: t.astype(jnp.bfloat16) if jnp.issubdtype(t.dtype, jnp.floating) else t)(jnp.asarray(a)))
    def _A_setup():
        B, S, D, H = 1, 2048, 576, 32
        return {
            "x": _w((lambda *s: _rng.normal(s) * 0.05)(B, S, D)),
            "wqkv": _w((lambda *s: _rng.normal(s) * 0.05)(D, 3 * D)),
            "wo": _w((lambda *s: _rng.normal(s) * 0.05)(D, D)),
        }
    _A_in = _A_setup()

    def _B_setup():
        B, S, D, F = 1, 2048, 576, 4608
        return {
            "x": _w((lambda *s: _rng.normal(s) * 0.05)(B, S, D)),
            "w1": _w((lambda *s: _rng.normal(s) * 1.6)(D, F) * (D ** -0.5)),
            "b1": _w((lambda *s: _rng.normal(s) * 0.05)(F)),
            "w2": _w((lambda *s: _rng.normal(s) * 0.05)(F, D) * (F ** -0.5)),
        }
    _B_in = _B_setup()

    return {
        "A_x": _A_in["x"],
        "A_wqkv": _A_in["wqkv"],
        "A_wo": _A_in["wo"],
        "B_x": _B_in["x"],
        "B_w1": _B_in["w1"],
        "B_b1": _B_in["b1"],
        "B_w2": _B_in["w2"],
    }

def reference(A_x, A_wqkv, A_wo, B_x, B_w1, B_b1, B_w2):
    def _A_ref(x, wqkv, wo):
        B, S, D = x.shape
        H = 32
        Dh = D // H
        qkv = (lambda x, *d: x.transpose(*d))((x @ wqkv).reshape(B, S, 3, H, Dh), 2, 0, 3, 1, 4)
        q, k, v = qkv[0], qkv[1], qkv[2]
        scores = jnp.einsum("bhqd,bhkd->bhqk", q, k) * (Dh ** -0.5)
        p = _softmax(scores, axis=-1)
        o = jnp.einsum("bhqk,bhkd->bhqd", p, v)
        return (lambda x, *d: x.transpose(*d))(o, 0, 2, 1, 3).reshape(B, S, D) @ wo

    def _B_ref(x, w1, b1, w2):
        h = jnp.einsum("bsd,df->bsf", x, w1) + b1
        sp = jnp.log1p(jnp.exp(-jnp.abs(h))) + jnp.where(h > 0, h, jnp.zeros_like(h))
        act = h * jnp.tanh(sp)
        return jnp.einsum("bsf,fd->bsd", act, w2)

    x = A_x
    h = x + _A_ref(_layernorm(x, axis=-1), A_wqkv, A_wo)
    h2 = h + _B_ref(_layernorm(h, axis=-1), B_w1, B_b1, B_w2)
    return h2
```

```python
import jax
import jax.numpy as jnp
import jax.experimental.pallas as pl
import jax.experimental.pallas.tpu as pltpu

S = 2048
D = 576
H = 32
DH = 18
F = 4608
HPG = 7
NG = 5
GW = NG * 128
VP = 32
VW = H * VP
TQ = 256
FC = 512
EPS = 1e-5
KC = 256
LOG2E = 1.4426950408889634


def _ln(x):
    m = jnp.mean(x, axis=-1, keepdims=True)
    xc = x - m
    v = jnp.mean(xc * xc, axis=-1, keepdims=True)
    return xc * jax.lax.rsqrt(v + EPS)


def _kernel(x_ref, wqkv_ref, wo_ref, w1_hbm, b1_ref, w2_hbm, o_ref,
            k_scr, vt_scr, qt_scr, ot_scr, sA, sB, wq_ref, wk_ref, wop_ref,
            w1_ref, w2_ref, sem):
    i = pl.program_id(0)
    cp1 = pltpu.make_async_copy(w1_hbm, w1_ref, sem.at[0])
    cp2 = pltpu.make_async_copy(w2_hbm, w2_ref, sem.at[1])

    @pl.when(i == 0)
    def _():
        cp1.start()
        cp2.start()

    @pl.when(i == 0)
    def _():
        wq_ref[...] = jnp.zeros(wq_ref.shape, wq_ref.dtype)
        wk_ref[...] = jnp.zeros(wk_ref.shape, wk_ref.dtype)
        GC = HPG * DH
        for g in range(NG):
            n = min(GC, D - g * GC)
            wq_ref[:, g * 128:g * 128 + n] = wqkv_ref[:, g * GC:g * GC + n]
            wk_ref[:, g * 128:g * 128 + n] = wqkv_ref[:, D + g * GC:D + g * GC + n]
        wop_ref[...] = jnp.zeros(wop_ref.shape, wop_ref.dtype)
        wo32 = wo_ref[...].astype(jnp.float32)
        for h in range(H):
            wop_ref[h * VP:h * VP + DH, :] = wo32[h * DH:(h + 1) * DH, :].astype(jnp.bfloat16)
        vt_scr[...] = jnp.zeros(vt_scr.shape, vt_scr.dtype)

        def body(c, carry):
            r = pl.multiple_of(c * TQ, TQ)
            xn = _ln(x_ref[:, pl.ds(r, TQ)].astype(jnp.float32).T).astype(jnp.bfloat16)
            k_scr[pl.ds(r, TQ), :] = jnp.dot(
                xn, wk_ref[...], preferred_element_type=jnp.float32).astype(jnp.bfloat16)
            v = jnp.dot(xn, wqkv_ref[:, 2 * D:], preferred_element_type=jnp.float32)
            v = jnp.concatenate([v, jnp.zeros((TQ, GW - D), jnp.float32)], axis=1)
            vt = v.T
            for h in range(H):
                vt_scr[h * VP:h * VP + DH, pl.ds(r, TQ)] = (
                    vt[h * DH:(h + 1) * DH, :].astype(jnp.bfloat16))
            return carry
        jax.lax.fori_loop(0, S // TQ, body, 0)

    r0 = pl.multiple_of(i * TQ, TQ)
    xb = x_ref[:, pl.ds(r0, TQ)].astype(jnp.float32).T
    xn = _ln(xb).astype(jnp.bfloat16)
    q = jnp.dot(xn, wq_ref[...], preferred_element_type=jnp.float32) * (DH ** -0.5 * LOG2E)
    qt_scr[...] = q.T

    row = jax.lax.broadcasted_iota(jnp.int32, (128, TQ), 0)
    NC = S // KC

    def qm_of(h):
        g = h // HPG
        j = h - g * HPG
        off = pl.multiple_of(g * 128, 128)
        msk = (row >= j * DH) & (row < (j + 1) * DH)
        qm = jnp.where(msk, qt_scr[pl.ds(off, 128), :], 0.0).astype(jnp.bfloat16)
        return off, qm

    def stage(h_cur, s_cur, m_cur, h_nxt, s_nxt):
        if h_nxt is not None:
            off, qm = qm_of(h_nxt)
        if h_cur is not None:
            voff = pl.multiple_of(h_cur * VP, VP)
            l = jnp.zeros((1, TQ), jnp.float32)
            ot = jnp.zeros((VP, TQ), jnp.float32)
        m_nxt = None
        for c in range(NC):
            rows = pl.ds(c * KC, KC)
            if h_nxt is not None:
                st = jnp.dot(k_scr[rows, pl.ds(off, 128)], qm, preferred_element_type=jnp.float32)
                s_nxt[rows, :] = st
                mc = jnp.max(st, axis=0, keepdims=True)
                m_nxt = mc if m_nxt is None else jnp.maximum(m_nxt, mc)
            if h_cur is not None:
                p = jnp.exp2(s_cur[rows, :] - m_cur)
                l = l + jnp.sum(p, axis=0, keepdims=True)
                ot = ot + jnp.dot(vt_scr[pl.ds(voff, VP), rows], p.astype(jnp.bfloat16),
                                  preferred_element_type=jnp.float32)
        if h_cur is not None:
            ot_scr[pl.ds(voff, VP), :] = ot / l
        return m_nxt

    mA = stage(None, None, None, 0, sA)

    def head_body(it, mA):
        h = it * 2
        mB = stage(h, sA, mA, h + 1, sB)
        return stage(h + 1, sB, mB, jnp.minimum(h + 2, H - 1), sA)
    jax.lax.fori_loop(0, H // 2, head_body, mA)

    attn = jax.lax.dot_general(ot_scr[...].astype(jnp.bfloat16), wop_ref[...],
                               (((0,), (0,)), ((), ())),
                               preferred_element_type=jnp.float32)
    h1 = xb + attn

    @pl.when(i == 0)
    def _():
        cp1.wait()
        cp2.wait()

    hn = _ln(h1).astype(jnp.bfloat16)
    acc = h1
    for c in range(F // FC):
        t = jnp.dot(hn, w1_ref[:, c * FC:(c + 1) * FC], preferred_element_type=jnp.float32)
        t = t + b1_ref[:, c * FC:(c + 1) * FC].astype(jnp.float32)
        sp = jnp.log1p(jnp.exp(-jnp.abs(t))) + jnp.where(t > 0, t, 0.0)
        a = t * jnp.tanh(sp)
        acc = acc + jax.lax.dot_general(a.astype(jnp.bfloat16), w2_ref[:, c * FC:(c + 1) * FC],
                                        (((1,), (1,)), ((), ())),
                                        preferred_element_type=jnp.float32)
    o_ref[...] = acc.T.astype(o_ref.dtype)


@jax.jit
def pallas_sequential_preLN__mha_block__dense_activation_mish__prompt_kernel(
    A_x, A_wqkv, A_wo, B_x, B_w1, B_b1, B_w2,
):
    x = A_x.reshape(S, D).T
    b1 = B_b1.reshape(1, F)

    full = lambda shape: pl.BlockSpec(shape, lambda i: (0,) * len(shape))
    out = pl.pallas_call(
        _kernel,
        grid=(S // TQ,),
        in_specs=[
            full((D, S)), full((D, 3 * D)), full((D, D)),
            pl.BlockSpec(memory_space=pl.ANY), full((1, F)),
            pl.BlockSpec(memory_space=pl.ANY),
        ],
        out_specs=pl.BlockSpec((D, TQ), lambda i: (0, i)),
        out_shape=jax.ShapeDtypeStruct((D, S), A_x.dtype),
        scratch_shapes=[
            pltpu.VMEM((S, GW), jnp.bfloat16),
            pltpu.VMEM((VW, S), jnp.bfloat16),
            pltpu.VMEM((GW, TQ), jnp.float32),
            pltpu.VMEM((VW, TQ), jnp.float32),
            pltpu.VMEM((S, TQ), jnp.float32),
            pltpu.VMEM((S, TQ), jnp.float32),
            pltpu.VMEM((D, GW), jnp.bfloat16),
            pltpu.VMEM((D, GW), jnp.bfloat16),
            pltpu.VMEM((VW, D), jnp.bfloat16),
            pltpu.VMEM((D, F), jnp.bfloat16),
            pltpu.VMEM((D, F), jnp.bfloat16),
            pltpu.SemaphoreType.DMA((2,)),
        ],
        compiler_params=pltpu.CompilerParams(
            dimension_semantics=("arbitrary",),
            vmem_limit_bytes=100 * 1024 * 1024,
        ),
    )(x, A_wqkv, A_wo, B_w1, b1, B_w2.T)
    return out.T.reshape(1, S, D)
```
